```python
import os as _os
_os.environ.setdefault("JAX_PLATFORMS", "cpu")
import jax
import jax.numpy as jnp

def _softmax(x, axis=-1):
    return jax.nn.softmax(x, axis=axis)
def _gelu(x):
    return jax.nn.gelu(x, approximate=True)
def _silu(x):
    return jax.nn.silu(x)
def _sigmoid(x):
    return jax.nn.sigmoid(x)
def _layernorm(x, axis=-1, eps=1e-5):
    m = jnp.mean(x, axis=axis, keepdims=True)
    v = jnp.var(x, axis=axis, keepdims=True)
    return (x - m) / jnp.sqrt(v + eps)
def _scatter_add(tgt, idx, src, axis=0):
    return tgt.at[idx].add(src)
def _segment_sum(src, seg, n):
    return jax.ops.segment_sum(src, seg, n)
class _Rng:
    def __init__(self, key):
        self._k = key
    def _next(self):
        self._k, sub = jax.random.split(self._k)
        return sub
    def normal(self, shape):
        return jax.random.normal(self._next(), shape, dtype=jnp.bfloat16)
    def randint(self, lo, hi, shape):
        return jax.random.randint(self._next(), shape, lo, hi, dtype=jnp.int32)
    def uniform(self, shape, lo=0.0, hi=1.0):
        return jax.random.uniform(self._next(), shape, jnp.bfloat16, lo, hi)
    def permutation(self, n):
        return jax.random.permutation(self._next(), n)


kernel_name = 'sequential_preLN__ssm_conv_h3__mixer_channel_mlp__prompt'

def setup_inputs():
    _rng = _Rng(jax.random.key(int.from_bytes(__import__("os").urandom(4), "little")))
    _w = (lambda a: (lambda t: t.astype(jnp.bfloat16) if jnp.issubdtype(t.dtype, jnp.floating) else t)(jnp.asarray(a)))
    def _A_setup():
        B, S, D = 1, 2048, 448
        ks = 4
        return {
            "q": _w((lambda *s: _rng.normal(s) * 0.05)(B, S, D)),
            "k": _w((lambda *s: _rng.normal(s) * 0.05)(B, S, D)),
            "v": _w((lambda *s: _rng.normal(s) * 0.05)(B, S, D)),
            "shift_k": _w((lambda *s: _rng.normal(s) * 0.05)(D, ks) * 0.5),
            "ssm_k": _w((lambda *s: _rng.normal(s) * 0.05)(D, S) * (1.0 / S ** 0.5)),
            "ssm_D": _w((lambda *s: _rng.normal(s) * 0.05)(D)),
        }
    _A_in = _A_setup()

    def _B_setup():
        B, S, D, F = 1, 2048, 448, 1792
        return {
            "x": _w((lambda *s: _rng.normal(s) * 0.05)(B, S, D)),
            "w1": _w((lambda *s: _rng.normal(s) * 0.2)(D, F) * (D ** -0.5)),
            "b1": _w((lambda *s: _rng.normal(s) * 0.2)(F)),
            "w2": _w((lambda *s: _rng.normal(s) * 0.2)(F, D) * (F ** -0.5)),
            "b2": _w((lambda *s: _rng.normal(s) * 0.05)(D)),
        }
    _B_in = _B_setup()

    return {
        "A_q": _A_in["q"],
        "A_k": _A_in["k"],
        "A_v": _A_in["v"],
        "A_shift_k": _A_in["shift_k"],
        "A_ssm_k": _A_in["ssm_k"],
        "A_ssm_D": _A_in["ssm_D"],
        "B_x": _B_in["x"],
        "B_w1": _B_in["w1"],
        "B_b1": _B_in["b1"],
        "B_w2": _B_in["w2"],
        "B_b2": _B_in["b2"],
    }

def reference(A_q, A_k, A_v, A_shift_k, A_ssm_k, A_ssm_D, B_x, B_w1, B_b1, B_w2, B_b2):
    def _A_ref(q, k, v, shift_k, ssm_k, ssm_D):
        B, S, D = q.shape
        ks = shift_k.shape[-1]
        k_pad = jnp.pad(k, ((0, 0), (ks - 1, 0), (0, 0)))
        k_shift = jnp.zeros_like(k)
        for t in range(ks):
            k_shift = k_shift + k_pad[:, t:t + S, :] * shift_k[:, ks - 1 - t][None, None, :]
        kv = k_shift * v
        L = 2 * S
        kv_pad = jnp.pad(kv, ((0, 0), (0, S), (0, 0)))
        kf_pad = jnp.pad(ssm_k, ((0, 0), (0, S)))
        kv_f = (lambda x, axes=(-2,-1): jnp.fft.rfft2(x.astype(jnp.float32), axes=axes))(kv_pad[:, None, :, :], axes=(1, 2))
        kf_f = (lambda x, axes=(-2,-1): jnp.fft.rfft2(x.astype(jnp.float32), axes=axes))(kf_pad[:, None, :], axes=(1, 2))
        kf_f = (lambda x, *d: x.transpose(*d))(kf_f, 1, 2, 0)
        y_f = kv_f * kf_f[None, :, :, :]
        y = (lambda x, s, axes=(-2,-1): jnp.fft.irfft2(x, s=s, axes=axes).astype(jnp.bfloat16))(y_f, (1, L), axes=(1, 2))[:, 0, :S, :]
        y = y + kv * ssm_D[None, None, :]
        return q * y

    def _B_ref(x, w1, b1, w2, b2):
        y = _layernorm(x, axis=-1)
        h = _gelu(jnp.einsum("bsd,df->bsf", y, w1) + b1)
        return jnp.einsum("bsf,fd->bsd", h, w2) + b2

    x = A_q
    h = x + _A_ref(_layernorm(x, axis=-1), A_k, A_v, A_shift_k, A_ssm_k, A_ssm_D)
    h2 = h + _B_ref(_layernorm(h, axis=-1), B_w1, B_b1, B_w2, B_b2)
    return h2
```

```python
import numpy as np
import jax
import jax.numpy as jnp
import jax.experimental.pallas as pl
import jax.experimental.pallas.tpu as pltpu

S, D, F = 2048, 448, 1792
T = 128
TB = 256
NS = S // TB
KA = D + 16
EPS = 1e-5
C0 = 0.7978845608028654
C1 = C0 * 0.044715
f32 = jnp.float32
bf16 = jnp.bfloat16
u32 = jnp.uint32
ZOFF = 4 * (NS + 1)
POFF = ZOFF + 2 * (NS + 1)
DOFF = POFF + 2
NLAST = 6
TAB_S = NS * NLAST * 4
AHEAD = 4
LAT = 160
PF = 52.0
PG = 27.0
PQ = 42.0
P16 = 32.0
PP = 34.0
P32 = 54.0
PD = 38.0
PLN = 30.0
GAP = 90.0
NR1 = 4
PLNT = 22.0
NRT = 5
RCL = 32
PT16 = 32.0
PD1 = 32.0
PK1 = 38.0
OSPL = 320
TX0 = 100.0
GX = 0.0
TY0 = 0.0
TZ0 = 0.0
GZ = 0.0
PZ0 = 38.0
PZ1 = 50.0
T0 = 80.0
PL4 = 0.0
G1 = 0.0
G2 = 0.0
PQB = 48.0
TG = -250.0
PGB = 30.0
XG = 13
PX1 = 50.0
PX2 = 44.0
TL1 = 700.0


def _tables():
    todo = {(c, j) for c in range(NS) for j in range(1, NS) if c + j < NS} - {(0, 1)}
    tab = np.zeros((NS, NLAST, 4), np.int32)
    tab[:, :] = (0, 1, NS, 0)
    half = None
    for r in range(2, NS):
        avail = sorted((p for p in todo if p[0] < r and p[1] <= r), key=lambda p: (p[0] + p[1], p[0]))
        nfull = 4 if r < NS - 1 else NLAST
        for i, (c, j) in enumerate(avail[:nfull]):
            tab[r, i] = (c, j, c + j, 0)
            todo.remove((c, j))
        if r < NS - 1:
            if half is not None:
                assert sum(half) >= r
                tab[r, 4] = (*half, sum(half), D // 2)
                half = None
            elif len(avail) > nfull and r < NS - 2:
                half = avail[nfull]
                tab[r, 4] = (*half, sum(half), 0)
                todo.remove(half)
        assert all(c + j > r for c, j in todo)
    assert not todo and half is None
    return np.concatenate([tab.reshape(-1), np.array([0, 0, 0, POFF, DOFF, 1, NS, 2, 2, 4], np.int32)])


def _cmul(ar, ai, br, bi):
    return ar * br - ai * bi, ar * bi + ai * br


def _colsum(acc):
    return jnp.broadcast_to(jnp.sum(acc, axis=0, keepdims=True) * (1.0 / D), acc.shape)


def _as_f32(x_u32):
    return jax.lax.bitcast_convert_type(x_u32, f32)


def _add(acc, t):
    return t if acc is None else acc + t


def _kernel(q_hbm, k_hbm, v_hbm, g_hbm, w1_hbm, w2t_hbm, tab_hbm, sk_hbm, dd_hbm, b1_hbm, b2_hbm,
            o_hbm,
            q_s, kin_s, g_s, w1r_s, w2r_s, o_s,
            w1t_s, w2t_s, b2_s, u_s, ucur_s, graw_s, gz_s, w_s, kv_s, ly_s, act_s, hc_s, fwd_ref, inv_ref, xa_s,
            tab_ref, sk_ref, dd_ref, b1_ref, b2_ref, sem):
    oq = {}

    def cols(i):
        if isinstance(i, int):
            return slice(i * TB, (i + 1) * TB)
        return pl.ds(pl.multiple_of(i * TB, TB), TB)

    def sq(i):
        if isinstance(i, int) and i < 2:
            return NS + 1 if i == 0 else 2
        return i + 1

    def cp_q(i):
        return pltpu.make_async_copy(q_hbm.at[:, cols(i)], q_s.at[i], sem.at[sq(i)])

    def cp_k(i):
        return pltpu.make_async_copy(k_hbm.at[:, cols(i)], kin_s.at[2 * i + 2], sem.at[i])

    def cp_v(i):
        return pltpu.make_async_copy(v_hbm.at[:, cols(i)], kin_s.at[2 * i + 3], sem.at[i])

    def cp_g(i):
        return pltpu.make_async_copy(g_hbm.at[:, cols(i)], g_s.at[i], sem.at[NS + 5 if isinstance(i, int) and i == 0 else i])

    def cp_o(i):
        return pltpu.make_async_copy(o_s.at[i], o_hbm.at[:, cols(i)], sem.at[NS + 6])

    def cp_w1(i):
        return pltpu.make_async_copy(w1_hbm.at[:, cols(i)], w1r_s.at[:, cols(i)], sem.at[NS + 2 if i < 3 else (NS + 3 if i < 5 else NS + 7)])

    def cp_w2(i):
        return pltpu.make_async_copy(w2t_hbm.at[:, cols(i)], w2r_s.at[:, cols(i)], sem.at[1 if i < 2 else (NS + 4 if i < 4 else 2)])

    small = dict(tab=(tab_hbm, tab_ref), sk=(sk_hbm, sk_ref), dd=(dd_hbm, dd_ref), b1=(b1_hbm, b1_ref),
                 b2=(b2_hbm, b2_ref))

    def cp_s(name):
        return pltpu.make_async_copy(*small[name], sem.at[NS + 5])

    def col_bcast(row):
        return jnp.broadcast_to(row, (128, D)).T

    def init_taps():
        sk = sk_ref[...].astype(f32)
        for j in range(4):
            gz_s[POFF + j // 2, :, (j % 2) * T:(j % 2 + 1) * T] = col_bcast(sk[j:j + 1, :])

    def init_dft():
        def trig(rows, step):
            n = jax.lax.broadcasted_iota(jnp.int32, (rows, T), 0) * step
            f = jax.lax.broadcasted_iota(jnp.int32, (rows, T), 1)
            ang = (((2 * f + 1) * n) & (4 * T - 1)).astype(f32) * (np.pi / (2 * T))
            return jnp.cos(ang), jnp.sin(ang)

        cb, sb = trig(8, 1)
        ca, sa = trig(T // 8, 8)
        cs, sn = [], []
        for a in range(T // 8):
            c1 = jnp.broadcast_to(ca[a:a + 1], (8, T))
            s1 = jnp.broadcast_to(sa[a:a + 1], (8, T))
            cs.append(c1 * cb - s1 * sb)
            sn.append(-(s1 * cb + c1 * sb))
        c = jnp.concatenate(cs, axis=0)
        sn = jnp.concatenate(sn, axis=0)
        fwd_ref[:, :T] = pltpu.bitcast(c.astype(bf16), u32)
        fwd_ref[:, T:] = pltpu.bitcast(sn.astype(bf16), u32)
        inv_ref[:T // 2, :] = pltpu.bitcast((c.T * (1.0 / T)).astype(bf16), u32)
        inv_ref[T // 2:, :] = pltpu.bitcast((sn.T * (1.0 / T)).astype(bf16), u32)

    def init_const():
        rows = jax.lax.broadcasted_iota(jnp.int32, (16, TB), 0)
        xa_s[D // 2:, :] = pltpu.bitcast(jnp.where(rows == 0, 1.0, 0.0).astype(bf16), u32)

    def zero_z(lo, hi, t0, t1):
        n = (hi - lo) * 7
        for i in range(n):
            z = jnp.where(oq["zeros"][0] != 0, mxu_tok(t0 + (t1 - t0) * i / n), 0.0)
            z = jnp.concatenate([z, z], axis=1)
            gz_s[ZOFF + lo + i // 7, (i % 7) * 64:(i % 7 + 1) * 64, :] = jnp.concatenate([z] * 8, axis=0)

    def init_w1(lo, hi):
        b1 = b1_ref[...].astype(f32).reshape(1, F)[:, lo:hi]
        rows = jax.lax.broadcasted_iota(jnp.int32, (16, hi - lo), 0)
        ext = jnp.where(rows == 0, jnp.broadcast_to(b1, (16, hi - lo)), 0.0).astype(bf16)
        waug = jnp.concatenate([w1r_s[:, lo:hi], ext], axis=0)
        w1t_s[lo // 2:hi // 2, :] = pltpu.bitcast(waug.T, u32)

    def init_w2(lo, hi):
        w2t_s[:, lo:hi] = pltpu.bitcast(w2r_s[:, lo:hi], u32)

    stream = []

    def mxu_tok(t):
        r = max(int(t) - LAT, 0) // 8 * 8
        for x in stream:
            if r < x.shape[0]:
                return x[r:r + 8]
            r -= x.shape[0]
        return stream[-1][-8:]

    free = [False]

    def tok_gz(x):
        if not free[0]:
            gz_s[oq["doff"], 0:8, :T] = x

    def tok_kin(x):
        if not free[0]:
            kin_s[oq["kdum"], 0:8, :T] = pltpu.bitcast(x, bf16)[0:8]

    def tok_q(x, force=False):
        if force or not free[0]:
            q_s[oq["qdum"], 0:8, :T] = pltpu.bitcast(x, bf16)[0:8]

    def tok_u(x):
        if not free[0]:
            ucur_s[oq["udum"], 0:8, :T] = x

    def tok_r(x):
        if not free[0]:
            graw_s[oq["rdum"], 0:8, :T] = x

    def tok_ly(x, force=False):
        if force or not free[0]:
            ly_s[oq["ldum"], 0:8, :T] = x

    def cplx(ref, e, rs):
        return ref[e, rs, :T], ref[e, rs, T:]

    def put(ref, e, rs, re, im):
        ref[e, rs, :T] = re
        ref[e, rs, T:] = im

    def fwd(tok=False):
        a = kv_s[...]
        if tok:
            tok_gz(_as_f32(a[0:8, :T]))
            tok_kin(_as_f32(a[0:8, :T]))
        for b in range(2):
            u = jnp.dot(pltpu.bitcast(a[:, b * T:(b + 1) * T], bf16), pltpu.bitcast(fwd_ref[...], bf16),
                        preferred_element_type=f32)
            ucur_s[b] = u
        stream.append(u[:, :T])

    def gdft(jsrc, buf):
        for b in range(2):
            u = jnp.dot(g_s[jsrc, :, b * T:(b + 1) * T], pltpu.bitcast(fwd_ref[...], bf16), preferred_element_type=f32)
            graw_s[2 * buf + b] = u
        stream.append(u[:, :T])

    def inv():
        w = w_s[...]
        for b in range(2):
            y = jnp.dot(pltpu.bitcast(w[:, 2 * b * T:2 * (b + 1) * T], bf16), pltpu.bitcast(inv_ref[...], bf16),
                        preferred_element_type=f32)
            ly_s[0, :, b * T:(b + 1) * T] = y
        stream.append(y)

    def m1(lo=0, hi=F):
        rh = slice(lo // 2, hi // 2)
        h = jnp.dot(pltpu.bitcast(w1t_s[rh, :], bf16), pltpu.bitcast(xa_s[...], bf16),
                    preferred_element_type=f32)
        stream.append(h[:, :T])
        stream.append(h[:, T:])
        u = h * (C0 + C1 * (h * h))
        act_s[rh, :] = pltpu.bitcast((h + h * jnp.tanh(u)).astype(bf16), u32)

    def m2(i, lo, hi):
        KG = 512
        for n in range(lo, hi):
            kg, b = n // 2, n % 2
            if kg < 3:
                cs = slice(b * T, (b + 1) * T)
                a = act_s[kg * KG // 2:(kg + 1) * KG // 2, cs]
                p = jnp.dot(pltpu.bitcast(w2t_s[:, kg * KG:(kg + 1) * KG], bf16), pltpu.bitcast(a, bf16),
                            preferred_element_type=f32)
                stream.append(p)
                if kg == 0:
                    hc_s[oq["zeros"][0], :, cs] = p + (ly_s[1, :, cs] * 2.0 + b2_s[0])
                else:
                    hc_s[oq["zeros"][kg % 2], :, cs] += p
            else:
                p = jnp.dot(pltpu.bitcast(w2t_s[:, 3 * KG:], bf16), pltpu.bitcast(act_s[3 * KG // 2:, :], bf16),
                            preferred_element_type=f32)
                stream.append(p[:, :T])
                o_s[i] = ((hc_s[oq["zeros"][1]] + p) * 0.5).astype(bf16)

    def slot_part(c, j, a, r, rc, first=False, base=None):
        rs = slice(r, r + rc) if base is None else pl.ds(pl.multiple_of(base + r, 16), rc)

        def load():
            return ([cplx(u_s, 3 * c + e, rs) for e in range(3)],
                    [cplx(gz_s, 4 * j + e, rs) for e in range(3)],
                    [(None, None) if first else cplx(gz_s, ZOFF + 2 * a + e, rs) for e in range(2)])

        def finish(st):
            (u0, u1, us), (g0, ga, gb), (z0, z1) = st
            pr, pi = _cmul(*g0, *us)
            ar, ai = _cmul(*ga, *u1)
            br, bi = _cmul(*gb, *u0)
            put(gz_s, ZOFF + 2 * a, rs, _add(z0[0], pr + ar), _add(z0[1], pi + ai))
            last = _add(z1[1], pi + bi)
            put(gz_s, ZOFF + 2 * a + 1, rs, _add(z1[0], pr + br), last)
            return last[:8]

        return load, finish

    def kv_load(i, r):
        rs = slice(r, r + 16)
        lane = jax.lax.broadcasted_iota(jnp.int32, (8, T), 1)
        if isinstance(i, int) and i == 0:
            prev = [jnp.zeros((8, T), u32)] * 3
        else:
            kp = pltpu.bitcast(kin_s[2 * i, rs, T:], u32)
            prev = [pltpu.roll(kp, j, 1) for j in range(1, 4)]
        out = []
        for b in range(2):
            k32 = pltpu.bitcast(kin_s[2 * i + 2, rs, b * T:(b + 1) * T], u32)
            sh = [k32]
            rolled = []
            for j in range(1, 4):
                rr = pltpu.roll(k32, j, 1)
                rolled.append(rr)
                sh.append(jnp.where(lane < j, prev[j - 1], rr))
            prev = rolled
            out.append((sh, kin_s[2 * i + 3, rs, b * T:(b + 1) * T]))
        return out

    def kv_parts(i):
        rows = list(range(0, D, 16))
        pend = []

        def make(n):
            r = rows[n]
            rs = slice(r, r + 16)
            rh = slice(r // 2, r // 2 + 8)

            def load():
                if n == 0:
                    pend.extend(kv_load(i, rr) for rr in rows[:AHEAD])
                return [gz_s[(POFF if free[0] else oq["poff"]) + j // 2, rs, (j % 2) * T:(j % 2 + 1) * T] for j in range(4)]

            def finish(taps):
                loaded = pend.pop(0)
                res = []
                for b in range(2):
                    sh, v = loaded[b]
                    ks = pltpu.bitcast(sh[0], bf16).astype(f32) * taps[0]
                    for j in range(1, 4):
                        ks = ks + pltpu.bitcast(sh[j], bf16).astype(f32) * taps[j]
                    kv = ks * v.astype(f32)
                    kv_s[rh, b * T:(b + 1) * T] = pltpu.bitcast(kv.astype(bf16), u32)
                    res.append(kv)
                t = res[0] + res[1]
                t = t[:8] + t[8:]
                tok_gz(t)
                tok_kin(t)
                if n + AHEAD < len(rows):
                    pend.append(kv_load(i, rows[n + AHEAD]))
                return t

            return load, finish

        return [make(n) for n in range(len(rows))]

    def g_part(j, buf, r, first=False):
        rs = slice(r, r + 16)

        def load():
            st = [cplx(graw_s, 2 * buf, rs), cplx(graw_s, 2 * buf + 1, rs)]
            if not first:
                st += [cplx(graw_s, 2 * (1 - buf) + 1, rs), cplx(gz_s, 4 * (j - 1) + 3, rs)]
            return st

        def finish(st):
            lane = jax.lax.broadcasted_iota(jnp.int32, (16, T), 1)
            sgn = jnp.where(lane % 2 == 0, 1.0, -1.0).astype(f32)
            r0, r1 = st[0], st[1]
            gpr, gpi = r1[0] - sgn * r0[1], r1[1] + sgn * r0[0]
            put(gz_s, 4 * j + 3, rs, gpr, gpi)
            if first:
                put(gz_s, 4 * j, rs, r0[0] + b2_s[1, rs, :], r0[1])
                return gpi[:8]
            rm, gm = st[2], st[3]
            g0r, g0i = r0[0] - sgn * rm[1], r0[1] + sgn * rm[0]
            put(gz_s, 4 * j, rs, g0r, g0i)
            put(gz_s, 4 * j + 1, rs, gm[0] - g0r, gm[1] - g0i)
            last = gpi - g0i
            put(gz_s, 4 * j + 2, rs, gpr - g0r, last)
            tok_r(last[:8])
            return last[:8]

        return load, finish

    def pub_part(a, r):
        rs = slice(r, r + 16)

        def load():
            return [cplx(ucur_s, e, rs) for e in range(2)]

        def finish(st):
            u0, u1 = st
            put(u_s, 3 * a, rs, *u0)
            put(u_s, 3 * a + 1, rs, *u1)
            put(u_s, 3 * a + 2, rs, u0[0] + u1[0], u0[1] + u1[1])
            return u0[0][:8]

        return load, finish

    def diag_part(a, r, first=False):
        rs = slice(r, r + 16)
        rh = slice(r // 2, r // 2 + 8)

        def load():
            return ([cplx(ucur_s, e, rs) for e in range(2)],
                    [cplx(gz_s, (0 if free[0] else oq["gzero"]) + e, rs) for e in (0, 3)],
                    [(None, None) if first else cplx(gz_s, ZOFF + 2 * a + e, rs) for e in range(2)],
                    _as_f32(w_s[pl.ds(pl.multiple_of(oq["zeros"][0], 8), 8), :T]) if r and not free[0] else None)

        def finish(st):
            (u0, u1), (g0, gp), (z0, z1), prev = st
            ar, ai = _cmul(*u0, *g0)
            cr, ci = _cmul(*u0, *gp)
            dr, di = _cmul(*u1, *g0)
            w = [_add(z0[0], ar), _add(z0[1], ai), _add(z1[0], cr + dr), _add(z1[1], ci + di)]
            for n in range(4):
                w_s[rh, n * T:(n + 1) * T] = pltpu.bitcast(w[n].astype(bf16), u32)
            t = (w[0] + w[1]) + (w[2] + w[3])
            t = t[:8] + t[8:]
            if prev is not None:
                t = t + prev
            tok_gz(t)
            tok_u(t)
            return t

        return load, finish

    def qrows(i, r16):
        q = q_s[i, r16:r16 + 16, :].astype(f32)
        return q[:8], q[8:]

    def lnq_parts(i, out):
        st = {"acc": None}

        def make(kind, rows, last):
            def load():
                return [qrows(i, r) for r in rows]

            def finish(qs):
                for a, b in qs:
                    if kind == 1:
                        a, b = a - out["m"], b - out["m"]
                        st["acc"] = _add(st["acc"], a * a + b * b)
                    else:
                        st["acc"] = _add(st["acc"], a + b)
                t = st["acc"]
                if last:
                    t = _colsum(t)
                    if kind == 1:
                        t = jax.lax.rsqrt(t + EPS)
                    out["r" if kind else "m"] = t
                    st["acc"] = None
                t = t[:, :T] + t[:, T:]
                if not last:
                    tok_gz(t)
                tok_q(t, last)
                return t

            return load, finish

        rows = list(range(0, D, 16))
        p0 = [make(0, rows[n:n + 7], n + 7 == 28) for n in range(0, 28, 7)]
        p1 = [make(1, rows[n:n + 4], n + 4 == 28) for n in range(0, 28, 4)]
        return p0, p1

    def run(links, t=None):
        for parts, dur, rel in links:
            if t is not None and t > LAT:
                x = mxu_tok(t)
                tok_gz(x)
                for fn in rel:
                    fn(x)
            sts = [p[0]() for p in parts]
            for p, st in zip(parts, sts):
                last = p[1](st)
            if t is not None:
                t += dur
        return t, last

    def ln_rest(i, m1_, r1, t0=None, pln=PLN):
        clock = [t0]

        def pace(x, q=False, dt=pln, force=None):
            x = x[:, :T] + x[:, T:]
            for val in ([x] if t0 is None else [x, mxu_tok(clock[0] + dt)]):
                if q:
                    tok_q(val)
                tok_ly(val, dt != pln if force is None else force)
            if t0 is not None:
                clock[0] += dt

        acc = None
        for r in range(0, D, 16):
            a, b = qrows(i, r)
            ha = a + (a - m1_) * r1 * ly_s[0, r:r + 8, :]
            hb = b + (b - m1_) * r1 * ly_s[0, r + 8:r + 16, :]
            ly_s[1, r:r + 8, :] = ha
            ly_s[1, r + 8:r + 16, :] = hb
            acc = _add(acc, ha + hb)
            if r % 32 == 16 and r + 16 < D:
                pace(acc, q=True)
        m2_ = _colsum(acc)
        pace(m2_, dt=GAP)
        acc = None
        acc1 = None
        for r in range(0, D, 8):
            d = ly_s[1, r:r + 8, :] - m2_
            acc = _add(acc, d * d)
            acc1 = _add(acc1, d)
            if r % 64 == 56 and r + 8 < D:
                pace(acc + acc1, dt=pln + PL4, force=False)
        v2 = _colsum(acc)
        r2 = jax.lax.rsqrt(v2 + EPS)
        md = _colsum(acc1)
        m3_ = md * r2
        v3 = v2 * r2 * r2 - m3_ * m3_
        r3 = jax.lax.rsqrt(v3 + EPS)
        cc = m2_ + md
        rr = r2 * r3
        pace(rr, dt=GAP + 40)
        for r in range(0, D, 16):
            xa = (ly_s[1, r:r + 8, :] - cc) * rr
            xb = (ly_s[1, r + 8:r + 16, :] - cc) * rr
            xn = jnp.concatenate([xa, xb], axis=0).astype(bf16)
            xa_s[r // 2:r // 2 + 8, :] = pltpu.bitcast(xn, u32)
            if r % 96 == 80:
                pace(xb)

    R16 = list(range(0, D, 16))

    def block(s):
        del stream[:]
        nxt = s + 1
        buf = (s + 1) % 2
        fwd(True)
        gdft(nxt, buf)
        m1()
        m2(s - 1, 0, NR1)
        terms = [[tab_ref[(s * NLAST + i) * 4 + e] for e in range(4)] for i in range(5)]
        pos = [0]

        def slot(rc):
            i, r = divmod(pos[0], D)
            assert r + rc <= D
            pos[0] += rc
            return slot_part(*terms[i][:3], r, rc, base=terms[i][3] if i == 4 else None)

        stats = {}
        p0, p1 = lnq_parts(s, stats)
        links = []
        for p in kv_parts(nxt):
            links.append(([slot(16), p], PF, []))
        links[-1] = (links[-1][0], PF + G1, [])
        for p in p0:
            links.append(([slot(16), p], PQB, [tok_q]))
        for _ in range(3):
            links.append(([slot(16)], P16, []))
        for p in p1:
            links.append(([slot(16), p], PQB, [tok_q]))
        links[-1] = (links[-1][0], PQB + G2, [tok_q])
        for r in R16:
            links.append(([slot(16), pub_part(s, r)], PP, [tok_u]))
        while pos[0] < 4 * D + D // 2:
            links.append(([slot(RCL)], P32, []))
        links += [([diag_part(s, r)], PD, [tok_u]) for r in R16]
        t, last = run(links, T0)
        t_inv = sum(x.shape[0] for x in stream)
        inv()
        m2(s - 1, NR1, 7)
        run([([g_part(s + 1, buf, r)], PGB, [tok_r]) for r in R16], t_inv + TG)
        tok_q(mxu_tok(t_inv + D + LAT))
        ln_rest(s, stats["m"], stats["r"], t_inv + D + LAT)

    def tail():
        s = NS - 1 + oq["zeros"][0]
        del stream[:]
        fwd(True)
        m1()
        m2(NS - 2, 0, NRT)
        terms = [[tab_ref[((NS - 1) * NLAST + i) * 4 + e] for e in range(3)] for i in range(NLAST)]
        slots = [slot_part(*tm, r, 16) for tm in terms for r in R16]
        stats = {}
        p0, p1 = lnq_parts(s, stats)
        links = []
        for p in list(p0) + [None] * 3 + list(p1):
            links.append(([slots.pop(0)] + ([p] if p else []), PQ if p else P16, [tok_q] if p else []))
        links += [([p], PT16, []) for p in slots]
        links += [([diag_part(s, r)], PD, [tok_u]) for r in R16]
        run(links, 0.0)
        t_inv = sum(x.shape[0] for x in stream)
        inv()
        m2(NS - 2, NRT, 7)
        tok_q(mxu_tok(t_inv + D + LAT))
        ln_rest(s, stats["m"], stats["r"], t_inv + D + LAT, PLNT)
        cp_o(NS - 2).start()
        m1()
        m2_last(NS - 1)

    def cp_oh(i, b, lo=0, hi=D):
        return pltpu.make_async_copy(o_s.at[i, lo:hi, b * T:(b + 1) * T],
                                     o_hbm.at[lo:hi, i * TB + b * T:i * TB + (b + 1) * T], sem.at[NS + 6])

    def m2_last(i):
        KG = 512
        z = oq["zeros"]

        def part(kg, b):
            a = act_s[kg * KG // 2:(kg + 1) * KG // 2, b * T:(b + 1) * T]
            return jnp.dot(pltpu.bitcast(w2t_s[:, kg * KG:(kg + 1) * KG], bf16), pltpu.bitcast(a, bf16),
                           preferred_element_type=f32)

        c0, c1 = slice(0, T), slice(T, 2 * T)
        hc_s[z[0], :, c0] = part(0, 0) + (ly_s[1, :, c0] * 2.0 + b2_s[0])
        hc_s[z[1], :, c0] += part(1, 0)
        p = jnp.dot(pltpu.bitcast(w2t_s[:, 3 * KG:], bf16), pltpu.bitcast(act_s[3 * KG // 2:, :], bf16),
                    preferred_element_type=f32)
        hc_s[z[0], :, c0] += p[:, c0]
        hc_s[z[0], :, c1] = p[:, c1] + (ly_s[1, :, c1] * 2.0 + b2_s[0])
        o_s[i, :, c0] = ((hc_s[z[1], :, c0] + part(2, 0)) * 0.5).astype(bf16)
        cp_oh(i, 0).start()
        hc_s[z[1], :, c1] += part(0, 1)
        hc_s[z[0], :, c1] += part(1, 1)
        o = ((hc_s[z[1], :, c1] + part(2, 1)) * 0.5).astype(bf16)
        o_s[i, :OSPL, c1] = o[:OSPL]
        cp_oh(i, 1, 0, OSPL).start()
        o_s[i, OSPL:, c1] = o[OSPL:]
        cp_oh(i, 1, OSPL, D).start()

    def go(parts):
        run([(list(p) if isinstance(p, list) else [p], 0, []) for p in parts])

    cp_g(0).start()
    for name in small:
        cp_s(name).start()
    cp_k(0).start(); cp_v(0).start(); cp_q(0).start()
    for i in range(7):
        cp_w1(i).start()
    cp_k(1).start(); cp_v(1).start(); cp_g(1).start()
    for i in range(7):
        cp_w2(i).start()
    cp_q(1).start()
    cp_k(2).start(); cp_v(2).start(); cp_g(2).start()
    for i in range(3, NS):
        cp_q(i - 1).start(); cp_k(i).start(); cp_v(i).start(); cp_g(i).start()
    cp_q(NS - 1).start()
    free[0] = True
    init_const()
    init_dft()
    cp_g(0).wait()
    for name in small:
        cp_s(name).wait()
    oq["zeros"] = [tab_ref[TAB_S], tab_ref[TAB_S + 1]]
    for n, name in enumerate(["gzero", "poff", "doff", "kdum", "qdum", "ldum", "udum", "rdum"]):
        oq[name] = tab_ref[TAB_S + 2 + n]
    init_taps()
    b2_s[1] = col_bcast(dd_ref[...].astype(f32).reshape(1, D))
    b2_s[0] = col_bcast(b2_ref[...].astype(f32).reshape(1, D) * 2.0)
    gdft(0, 0)
    go([g_part(0, 0, r, True) for r in R16])
    cp_k(0).wait(); cp_v(0).wait()
    go(kv_parts(0))
    fwd()
    cp_q(0).wait()
    go([diag_part(0, r, True) for r in R16])
    inv()
    stats = {}
    p0, p1 = lnq_parts(0, stats)
    go(p0 + p1)
    ln_rest(0, stats["m"], stats["r"])
    for i in range(3):
        cp_w1(i).wait()
    del stream[:]
    init_w1(0, 3 * TB)
    m1(0, 2 * TB)
    free[0] = False
    run([([pub_part(0, r)], 20.0, [tok_u]) for r in R16], 400.0)
    free[0] = True
    for i in range(3, 5):
        cp_w1(i).wait()
    del stream[:]
    init_w1(3 * TB, 5 * TB)
    m1(2 * TB, 4 * TB)
    zero_z(4, 9, 300, 4 * TB)
    for i in range(5, 7):
        cp_w1(i).wait()
    del stream[:]
    init_w1(5 * TB, F)
    m1(4 * TB, F)
    zero_z(9, 2 * (NS + 1), 300, 6 * TB)
    cp_k(1).wait(); cp_v(1).wait(); cp_g(1).wait(); cp_w2(0).wait(); cp_w2(1).wait()
    free[0] = False
    del stream[:]
    gdft(1, 1)
    init_w2(0, 2 * TB)
    m2(0, 0, 2)
    kvp = kv_parts(1)
    gp = [g_part(1, 1, r) for r in R16]
    sp = [slot_part(0, 1, 1, r, 16, True) for r in R16]
    links = [([p], PK1, []) for p in kvp[:XG]]
    links += [([p, gp.pop(0)], PX1, [tok_r]) for p in kvp[XG:]]
    t, _ = run(links, TX0)
    fwd()
    run([([g, sp.pop(0)], PX2, [tok_r]) for g in gp], t + GX)
    cp_w2(2).wait(); cp_w2(3).wait()
    del stream[:]
    init_w2(2 * TB, 4 * TB)
    m2(0, 2, 4)
    links = []
    for r in R16:
        links.append(([diag_part(1, r)] + ([sp.pop(0)] if sp else []), PX1 if sp else PD1, [tok_u]))
    run(links, TY0)
    inv()
    for i in range(4, 7):
        cp_w2(i).wait()
    cp_k(2).wait(); cp_v(2).wait(); cp_g(2).wait(); cp_q(1).wait()
    del stream[:]
    gdft(2, 0)
    init_w2(4 * TB, F)
    m2(0, 4, 7)
    stats = {}
    p0, p1 = lnq_parts(1, stats)
    extra = list(p0) + [None, None] + list(p1)
    links = []
    for p, r in zip(kv_parts(2), R16):
        e = extra.pop(0) if extra else None
        links.append(([p, pub_part(1, r)] + ([e] if e else []), PZ1 if e else PZ0, [tok_u] + ([tok_q] if e else [])))
    t, _ = run(links, TZ0)
    run([([g_part(2, 0, r)], PG, [tok_r]) for r in R16], t + GZ)
    tok_q(mxu_tok(TL1))
    ln_rest(1, stats["m"], stats["r"], TL1)
    cp_o(0).start()

    def step(s, carry):
        cp_k(s + 1).wait(); cp_v(s + 1).wait(); cp_g(s + 1).wait(); cp_q(s).wait()
        block(s)
        cp_o(s - 1).start()
        return carry

    jax.lax.fori_loop(2, NS - 1, step, 0)
    cp_q(NS - 1).wait()
    tail()
    for i in range(NS - 1):
        cp_o(i).wait()
    cp_oh(NS - 1, 0).wait()
    cp_oh(NS - 1, 1, 0, OSPL).wait()
    cp_oh(NS - 1, 1, OSPL, D).wait()


@jax.jit
def pallas_sequential_preLN__ssm_conv_h3__mixer_channel_mlp__prompt_kernel(A_q, A_k, A_v, A_shift_k, A_ssm_k, A_ssm_D, B_x, B_w1, B_b1, B_w2, B_b2):
    qT = A_q[0].T
    kT = A_k[0].T
    vT = A_v[0].T
    hbm = pl.BlockSpec(memory_space=pl.ANY)
    tab = _tables()
    oT = pl.pallas_call(
        _kernel,
        in_specs=[hbm] * 11,
        out_specs=hbm,
        scratch_shapes=[
            pltpu.VMEM((NS + 1, D, TB), bf16),
            pltpu.VMEM((2 * NS + 2, D, TB), bf16),
            pltpu.VMEM((NS, D, TB), bf16),
            pltpu.VMEM((D, F), bf16),
            pltpu.VMEM((D, F), bf16),
            pltpu.VMEM((NS, D, TB), bf16),
            pltpu.VMEM((F // 2, KA), u32),
            pltpu.VMEM((D // 2, F), u32),
            pltpu.VMEM((2, D, 128), f32),
            pltpu.VMEM((3 * NS, D, 2 * T), f32),
            pltpu.VMEM((3, D, 2 * T), f32),
            pltpu.VMEM((5, D, 2 * T), f32),
            pltpu.VMEM((DOFF + 1, D, 2 * T), f32),
            pltpu.VMEM((D // 2, 4 * T), u32),
            pltpu.VMEM((D // 2, 2 * T), u32),
            pltpu.VMEM((3, D, TB), f32),
            pltpu.VMEM((F // 2, TB), u32),
            pltpu.VMEM((1, D, TB), f32),
            pltpu.VMEM((T // 2, 2 * T), u32), pltpu.VMEM((T, T), u32),
            pltpu.VMEM((KA // 2, TB), u32),
            pltpu.SMEM(tab.shape, jnp.int32),
            pltpu.VMEM((4, D), bf16), pltpu.VMEM((D,), bf16), pltpu.VMEM((F,), bf16), pltpu.VMEM((D,), bf16),
            pltpu.SemaphoreType.DMA((NS + 8,)),
        ],
        out_shape=jax.ShapeDtypeStruct((D, S), bf16),
        compiler_params=pltpu.CompilerParams(vmem_limit_bytes=110 * 1024 * 1024),
    )(qT, kT, vT, A_ssm_k, B_w1, B_w2.T, jnp.asarray(tab), A_shift_k.T, A_ssm_D, B_b1, B_b2)
    return oT.T[None]
```
